```python
import os as _os
_os.environ.setdefault("JAX_PLATFORMS", "cpu")
import jax
import jax.numpy as jnp

def _softmax(x, axis=-1):
    return jax.nn.softmax(x, axis=axis)
def _gelu(x):
    return jax.nn.gelu(x, approximate=True)
def _silu(x):
    return jax.nn.silu(x)
def _sigmoid(x):
    return jax.nn.sigmoid(x)
def _layernorm(x, axis=-1, eps=1e-5):
    m = jnp.mean(x, axis=axis, keepdims=True)
    v = jnp.var(x, axis=axis, keepdims=True)
    return (x - m) / jnp.sqrt(v + eps)
def _scatter_add(tgt, idx, src, axis=0):
    return tgt.at[idx].add(src)
def _segment_sum(src, seg, n):
    return jax.ops.segment_sum(src, seg, n)
class _Rng:
    def __init__(self, key):
        self._k = key
    def _next(self):
        self._k, sub = jax.random.split(self._k)
        return sub
    def normal(self, shape):
        return jax.random.normal(self._next(), shape, dtype=jnp.bfloat16)
    def randint(self, lo, hi, shape):
        return jax.random.randint(self._next(), shape, lo, hi, dtype=jnp.int32)
    def uniform(self, shape, lo=0.0, hi=1.0):
        return jax.random.uniform(self._next(), shape, jnp.bfloat16, lo, hi)
    def permutation(self, n):
        return jax.random.permutation(self._next(), n)


kernel_name = 'standalone__grn__sampling'

def setup_inputs():
    _rng = _Rng(jax.random.key(int.from_bytes(__import__("os").urandom(4), "little")))
    _w = (lambda a: (lambda t: t.astype(jnp.bfloat16) if jnp.issubdtype(t.dtype, jnp.floating) else t)(jnp.asarray(a)))
    B, S, D = 512, 32, 640
    return {
        "x": _w((lambda *s: _rng.normal(s) * 0.05)(B, S, D)),
        "g": _w((lambda *s: _rng.normal(s) * 0.1)(D) * 0.1),
        "b": _w((lambda *s: _rng.normal(s) * 0.1)(D) * 0.1),
    }

def reference(x, g, b):
    gx = jnp.sqrt((x * x).sum(axis=-2, keepdims=True))
    nx = gx / (gx.mean(axis=-1, keepdims=True) + 1e-6)
    return g * (x * nx) + b + x
```

```python
import jax
import jax.numpy as jnp
import jax.experimental.pallas as pl
import jax.experimental.pallas.tpu as pltpu

_STREAMS = 8
_READ_BOUNDS = (0, 12, 28, 63, 64)


def _grn_kernel(x_hbm, g_hbm, b_hbm, o_hbm, xbuf, obuf, gbuf, bbuf, rsem, wsem):
    streams = x_hbm.shape[0]
    bounds = _READ_BOUNDS
    groups = len(bounds) - 1

    def read(i):
        cols = pl.ds(bounds[i], bounds[i + 1] - bounds[i])
        return pltpu.make_async_copy(x_hbm.at[:, cols], xbuf.at[:, cols], rsem.at[i])

    def start_write(j):
        pltpu.make_async_copy(obuf.at[:, j], o_hbm.at[:, j], wsem).start()

    g_copy = pltpu.make_async_copy(g_hbm, gbuf, rsem.at[0])
    b_copy = pltpu.make_async_copy(b_hbm, bbuf, rsem.at[0])
    read(0).start()
    g_copy.start()
    b_copy.start()
    for i in range(1, groups):
        read(i).start()
    read(0).wait()
    g_copy.wait()
    b_copy.wait()

    g = gbuf[...].astype(jnp.float32).reshape(1, -1)
    b = bbuf[...].astype(jnp.float32).reshape(1, -1)

    def compute_column(j):
        for k in range(streams):
            x = xbuf[k, j].astype(jnp.float32)
            gx = jnp.sqrt(jnp.sum(x * x, axis=0, keepdims=True))
            nx = gx / (jnp.mean(gx, axis=-1, keepdims=True) + 1e-6)
            obuf[k, j] = (x * (g * nx + 1.0) + b).astype(obuf.dtype)

    def compute_and_write_column(j):
        compute_column(j)
        start_write(j)

    for i in range(groups):
        if i > 0:
            read(i).wait()
        if i == groups - 2:
            pl.loop(0, bounds[i])(start_write)
        body = compute_and_write_column if i >= groups - 2 else compute_column
        pl.loop(bounds[i], bounds[i + 1])(body)

    pltpu.make_async_copy(obuf, o_hbm, wsem).wait()


@jax.jit
def pallas_standalone__grn__sampling_kernel(
    x: jax.Array,
    g: jax.Array,
    b: jax.Array,
):
    B, S, D = x.shape
    shape = (_STREAMS, B // _STREAMS, S, D)
    out = pl.pallas_call(
        _grn_kernel,
        in_specs=[pl.BlockSpec(memory_space=pl.ANY)] * 3,
        out_specs=pl.BlockSpec(memory_space=pl.ANY),
        out_shape=jax.ShapeDtypeStruct(shape, x.dtype),
        scratch_shapes=[
            pltpu.VMEM(shape, x.dtype),
            pltpu.VMEM(shape, x.dtype),
            pltpu.VMEM(g.shape, g.dtype),
            pltpu.VMEM(b.shape, b.dtype),
            pltpu.SemaphoreType.DMA((len(_READ_BOUNDS) - 1,)),
            pltpu.SemaphoreType.DMA(()),
        ],
        compiler_params=pltpu.CompilerParams(vmem_limit_bytes=64 * 1024 * 1024),
    )(x.reshape(shape), g, b)
    return out.reshape(x.shape)
```

```python
import functools

import jax
import jax.numpy as jnp
import jax.experimental.pallas as pl
import jax.experimental.pallas.tpu as pltpu

_EPS = 1e-6

_LANES = 128
_TILE_ROWS = 8
_UNIT_ROWS = 16

_REGION_UNITS = 256
_STREAMS = 5
_PIECE_UNITS = 4
_TAIL_UNITS = 104
_STAGED_UNITS = 200
_SLABS_PER_BLOCK = 4
_UNROLL = 8


def _grn_kernel(
    x_hbm, g_hbm, b_hbm, o_hbm, xbuf, obuf, gbuf, bbuf, stage, sems,
    *, row_tiles, lane_tiles,
):
    n_units = xbuf.shape[0]
    n_blocks = obuf.shape[0] // _STREAMS
    batch_units = row_tiles * lane_tiles * _TILE_ROWS // _UNIT_ROWS
    slab_units = _STREAMS * _REGION_UNITS // _SLABS_PER_BLOCK
    slab_steps = slab_units // (batch_units * _UNROLL)
    n_slabs = n_blocks * _SLABS_PER_BLOCK
    block_writes = _REGION_UNITS // _PIECE_UNITS
    slab_writes = block_writes // _SLABS_PER_BLOCK
    head_slabs = 2 * _SLABS_PER_BLOCK
    assert slab_steps * batch_units * _UNROLL == slab_units
    assert head_slabs < n_slabs and _STAGED_UNITS <= slab_units

    sem_a, sem_b, sem_stage = sems.at[0], sems.at[1], sems.at[2]
    head_end = head_slabs * slab_units
    direct_end = n_units - _STAGED_UNITS
    body_end = direct_end - _TAIL_UNITS

    def read(lo, hi, sem):
        units = pl.ds(lo, hi - lo)
        return pltpu.make_async_copy(x_hbm.at[units], xbuf.at[units], sem)

    read_head = read(0, head_end, sem_a)
    read_g = pltpu.make_async_copy(g_hbm, gbuf, sem_a)
    read_b = pltpu.make_async_copy(b_hbm, bbuf, sem_a)
    read_tail = read(body_end, direct_end, sem_a)
    read_body = read(head_end, body_end, sem_b)
    staged = pl.ds(direct_end, _STAGED_UNITS)
    stage_in = pltpu.make_async_copy(x_hbm.at[staged], stage, sem_stage)
    stage_out = pltpu.make_async_copy(stage, xbuf.at[staged], sem_stage)

    def start_writes(first, count):
        @pl.loop(0, count)
        def _(i):
            t = first + i
            idx = (
                pl.ds((t // block_writes) * _STREAMS, _STREAMS),
                pl.ds((t % block_writes) * _PIECE_UNITS, _PIECE_UNITS),
            )
            pltpu.make_async_copy(obuf.at[idx], o_hbm.at[idx], sem_b).start()

    read_head.start()
    stage_in.start()
    read_g.start()
    read_b.start()
    read_body.start()
    read_head.wait()
    read_g.wait()
    read_b.wait()
    read_tail.start()

    def per_lane_tile(ref):
        v = ref[...].astype(jnp.float32).reshape(1, -1)
        return jnp.stack(
            [v[:, c * _LANES:(c + 1) * _LANES] for c in range(lane_tiles)]
        )

    g = per_lane_tile(gbuf)
    b = per_lane_tile(bbuf)
    obuf_units = obuf.reshape(xbuf.shape)

    def grn(n):
        units = pl.ds(n * batch_units, batch_units)
        x = xbuf[units].astype(jnp.float32)
        x = x.reshape(row_tiles, lane_tiles, _TILE_ROWS, _LANES)
        sumsq = jnp.sum(jnp.sum(x * x, axis=0), axis=1, keepdims=True)
        gx = jnp.sqrt(sumsq)
        gx_sum = jnp.sum(jnp.sum(gx, axis=0), axis=-1, keepdims=True)
        nx = gx / (gx_sum / (lane_tiles * _LANES) + _EPS)
        out = x * (g * nx + 1.0) + b
        out = out.reshape(batch_units, _UNIT_ROWS, _LANES)
        obuf_units[units] = out.astype(obuf.dtype)

    @pl.loop(0, n_slabs)
    def _(slab):
        @pl.when(slab == head_slabs)
        def _():
            stage_in.wait()
            stage_out.start()
            read_body.wait()
            start_writes(0, block_writes)
            read_tail.wait()

        @pl.when(slab >= head_slabs)
        def _():
            start_writes((slab - _SLABS_PER_BLOCK) * slab_writes, slab_writes)

        @pl.when(slab == n_slabs - 1)
        def _():
            stage_out.wait()

        @pl.loop(0, slab_steps)
        def _(i):
            step = slab * slab_steps + i
            for k in range(_UNROLL):
                grn(step * _UNROLL + k)

    start_writes((n_blocks - 1) * block_writes, block_writes)
    pltpu.make_async_copy(obuf, o_hbm, sem_b).wait()


@jax.jit
def pallas_standalone__grn__sampling_kernel(
    x: jax.Array,
    g: jax.Array,
    b: jax.Array,
):
    B, S, D = x.shape
    row_tiles, lane_tiles = S // _TILE_ROWS, D // _LANES
    n_units = B * S * D // (_UNIT_ROWS * _LANES)
    assert x.dtype.itemsize == 2
    assert S % _TILE_ROWS == 0 and D % _LANES == 0
    assert n_units % (_STREAMS * _REGION_UNITS) == 0
    in_shape = (n_units, _UNIT_ROWS, _LANES)
    out_shape = (n_units // _REGION_UNITS, _REGION_UNITS, _UNIT_ROWS, _LANES)

    x_units = x.reshape(B * row_tiles, _TILE_ROWS, lane_tiles, _LANES)
    x_units = x_units.transpose(0, 2, 1, 3).reshape(in_shape)

    out = pl.pallas_call(
        functools.partial(_grn_kernel, row_tiles=row_tiles, lane_tiles=lane_tiles),
        in_specs=[pl.BlockSpec(memory_space=pl.ANY)] * 3,
        out_specs=pl.BlockSpec(memory_space=pl.ANY),
        out_shape=jax.ShapeDtypeStruct(out_shape, x.dtype),
        scratch_shapes=[
            pltpu.VMEM(in_shape, x.dtype),
            pltpu.VMEM(out_shape, x.dtype),
            pltpu.VMEM(g.shape, g.dtype),
            pltpu.VMEM(b.shape, b.dtype),
            pltpu.SMEM((_STAGED_UNITS, _UNIT_ROWS, _LANES), x.dtype),
            pltpu.SemaphoreType.DMA((3,)),
        ],
        compiler_params=pltpu.CompilerParams(vmem_limit_bytes=64 * 1024 * 1024),
    )(x_units, g, b)

    out = out.reshape(B * row_tiles, lane_tiles, _TILE_ROWS, _LANES)
    return out.transpose(0, 2, 1, 3).reshape(B, S, D)
```

```python
import functools
import math

import jax
import jax.numpy as jnp
import jax.experimental.pallas as pl
import jax.experimental.pallas.tpu as pltpu

_EPS = 1e-6

_LANES = 128
_TILE_ROWS = 8
_UNIT_ROWS = 16

_REGION_UNITS = 256
_STREAMS = 5
_PIECE_UNITS = 4
_TAIL_UNITS = 104
_STAGED_UNITS = 240
_SLABS_PER_BLOCK = 4
_UNROLL = 8


def _divmod_pow2(i, n):
    assert n & (n - 1) == 0
    return i >> (n.bit_length() - 1), i & (n - 1)


def _grn_kernel(
    x_hbm, g_hbm, b_hbm, o_hbm, xbuf, obuf, gbuf, bbuf, stage, sems,
    *, row_tiles, lane_tiles,
):
    n_units = xbuf.shape[0]
    n_blocks = obuf.shape[0] // _STREAMS
    batch_units = row_tiles * lane_tiles * _TILE_ROWS // _UNIT_ROWS
    block_units = _STREAMS * _REGION_UNITS
    slab_units = block_units // _SLABS_PER_BLOCK
    slab_steps = slab_units // (batch_units * _UNROLL)
    n_slabs = n_blocks * _SLABS_PER_BLOCK
    block_writes = _REGION_UNITS // _PIECE_UNITS
    slab_writes = block_writes // _SLABS_PER_BLOCK
    assert slab_steps * batch_units * _UNROLL == slab_units
    assert n_blocks > 2 and _STAGED_UNITS <= slab_units

    sem_a, sem_b, sem_stage = sems.at[0], sems.at[1], sems.at[2]
    direct_end = n_units - _STAGED_UNITS
    body_end = direct_end - _TAIL_UNITS

    def read(lo, hi, sem):
        units = pl.ds(lo, hi - lo)
        return pltpu.make_async_copy(x_hbm.at[units], xbuf.at[units], sem)

    read_block0 = read(0, block_units, sem_a)
    read_g = pltpu.make_async_copy(g_hbm, gbuf, sem_a)
    read_b = pltpu.make_async_copy(b_hbm, bbuf, sem_a)
    read_block1 = read(block_units, 2 * block_units, sem_b)
    read_body = read(2 * block_units, body_end, sem_a)
    read_tail = read(body_end, direct_end, sem_b)
    staged = pl.ds(direct_end, _STAGED_UNITS)
    stage_in = pltpu.make_async_copy(x_hbm.at[staged], stage, sem_stage)
    stage_out = pltpu.make_async_copy(stage, xbuf.at[staged], sem_stage)

    def start_writes(first, count):
        @pl.loop(0, count)
        def _(i):
            block, piece = _divmod_pow2(first + i, block_writes)
            idx = (
                pl.ds(block * _STREAMS, _STREAMS),
                pl.ds(piece * _PIECE_UNITS, _PIECE_UNITS),
            )
            pltpu.make_async_copy(obuf.at[idx], o_hbm.at[idx], sem_a).start()

    read_block0.start()
    stage_in.start()
    read_g.start()
    read_b.start()
    read_block1.start()
    read_block0.wait()
    read_g.wait()
    read_b.wait()
    read_body.start()

    def per_lane_tile(ref):
        v = ref[...].astype(jnp.float32).reshape(1, -1)
        return jnp.stack(
            [v[:, c * _LANES:(c + 1) * _LANES] for c in range(lane_tiles)]
        )

    g = per_lane_tile(gbuf)
    b = per_lane_tile(bbuf)
    run = math.gcd(batch_units, _REGION_UNITS)

    def grn(n):
        first = n * batch_units
        x = xbuf[pl.ds(first, batch_units)].astype(jnp.float32)
        x = x.reshape(row_tiles, lane_tiles, _TILE_ROWS, _LANES)
        sumsq = jnp.sum(jnp.sum(x * x, axis=0), axis=1, keepdims=True)
        gx = jnp.sqrt(sumsq)
        gx_sum = jnp.sum(jnp.sum(gx, axis=0), axis=-1, keepdims=True)
        nx = gx / (gx_sum / (lane_tiles * _LANES) + _EPS)
        out = x * (g * nx + 1.0) + b
        out = out.reshape(batch_units, _UNIT_ROWS, _LANES).astype(obuf.dtype)
        for u in range(0, batch_units, run):
            region, offset = _divmod_pow2(first + u, _REGION_UNITS)
            obuf[region, pl.ds(offset, run)] = out[u:u + run]

    @pl.loop(0, n_slabs)
    def _(slab):
        @pl.when(slab == _SLABS_PER_BLOCK)
        def _():
            read_block1.wait()
            read_tail.start()

        @pl.when(slab == 2 * _SLABS_PER_BLOCK)
        def _():
            stage_in.wait()
            stage_out.start()
            read_body.wait()
            start_writes(0, block_writes)
            read_tail.wait()

        @pl.when(slab >= 2 * _SLABS_PER_BLOCK)
        def _():
            start_writes((slab - _SLABS_PER_BLOCK) * slab_writes, slab_writes)

        @pl.when(slab == n_slabs - 1)
        def _():
            stage_out.wait()

        @pl.loop(0, slab_steps)
        def _(i):
            step = slab * slab_steps + i
            for k in range(_UNROLL):
                grn(step * _UNROLL + k)

    start_writes((n_blocks - 1) * block_writes, block_writes)
    pltpu.make_async_copy(obuf, o_hbm, sem_a).wait()


@jax.jit
def pallas_standalone__grn__sampling_kernel(
    x: jax.Array,
    g: jax.Array,
    b: jax.Array,
):
    B, S, D = x.shape
    row_tiles, lane_tiles = S // _TILE_ROWS, D // _LANES
    n_units = B * S * D // (_UNIT_ROWS * _LANES)
    assert x.dtype.itemsize == 2
    assert S % _TILE_ROWS == 0 and D % _LANES == 0
    assert n_units % (_STREAMS * _REGION_UNITS) == 0
    in_shape = (n_units, _UNIT_ROWS, _LANES)
    out_shape = (n_units // _REGION_UNITS, _REGION_UNITS, _UNIT_ROWS, _LANES)

    x_units = x.reshape(B * row_tiles, _TILE_ROWS, lane_tiles, _LANES)
    x_units = x_units.transpose(0, 2, 1, 3).reshape(in_shape)

    out = pl.pallas_call(
        functools.partial(_grn_kernel, row_tiles=row_tiles, lane_tiles=lane_tiles),
        in_specs=[pl.BlockSpec(memory_space=pl.ANY)] * 3,
        out_specs=pl.BlockSpec(memory_space=pl.ANY),
        out_shape=jax.ShapeDtypeStruct(out_shape, x.dtype),
        scratch_shapes=[
            pltpu.VMEM(in_shape, x.dtype),
            pltpu.VMEM(out_shape, x.dtype),
            pltpu.VMEM(g.shape, g.dtype),
            pltpu.VMEM(b.shape, b.dtype),
            pltpu.SMEM((_STAGED_UNITS, _UNIT_ROWS, _LANES), x.dtype),
            pltpu.SemaphoreType.DMA((3,)),
        ],
        compiler_params=pltpu.CompilerParams(vmem_limit_bytes=64 * 1024 * 1024),
    )(x_units, g, b)

    out = out.reshape(B * row_tiles, lane_tiles, _TILE_ROWS, _LANES)
    return out.transpose(0, 2, 1, 3).reshape(B, S, D)
```
